```python
import jax
import jax.numpy as jnp

def _softmax(x, axis=-1):
    return jax.nn.softmax(x, axis=axis)
def _gelu(x):
    return jax.nn.gelu(x, approximate=True)
def _silu(x):
    return jax.nn.silu(x)
def _sigmoid(x):
    return jax.nn.sigmoid(x)
def _layernorm(x, axis=-1, eps=1e-5):
    m = jnp.mean(x, axis=axis, keepdims=True)
    v = jnp.var(x, axis=axis, keepdims=True)
    return (x - m) / jnp.sqrt(v + eps)
def _scatter_add(tgt, idx, src, axis=0):
    return tgt.at[idx].add(src)
def _segment_sum(src, seg, n):
    return jax.ops.segment_sum(src, seg, n)
class _Rng:
    def __init__(self, key):
        self._k = key
    def _next(self):
        self._k, sub = jax.random.split(self._k)
        return sub
    def normal(self, shape):
        return jax.random.normal(self._next(), shape, dtype=jnp.bfloat16)
    def randint(self, lo, hi, shape):
        return jax.random.randint(self._next(), shape, lo, hi, dtype=jnp.int32)
    def uniform(self, shape, lo=0.0, hi=1.0):
        return jax.random.uniform(self._next(), shape, jnp.bfloat16, lo, hi)
    def permutation(self, n):
        return jax.random.permutation(self._next(), n)


kernel_name = 'recurrent_scan__sliding_block_cached__mixer_s_mlp__decode'

def _fwd_setup_inputs():
    _rng = _Rng(jax.random.key(int.from_bytes(__import__("os").urandom(4), "little")))
    _w = (lambda a: (lambda t: t.astype(jnp.bfloat16) if jnp.issubdtype(t.dtype, jnp.floating) else t)(jnp.asarray(a)))
    def _A_setup():
        B, Sq, D = 4, 1, 512
        Hq, Hkv, Sk, Dh = 32, 8, 8192, 128
        assert Hq % Hkv == 0, (Hq, Hkv)
        return {
            "x": _w((lambda *s: _rng.normal(s) * 0.05)(B, Sq, D)),
            "k_cache": _w((lambda *s: _rng.normal(s) * 0.05)(B, Hkv, Sk, Dh)),
            "v_cache": _w((lambda *s: _rng.normal(s) * 0.05)(B, Hkv, Sk, Dh)),
            "wq": _w((lambda *s: _rng.normal(s) * 0.05)(D, Hq * Dh) * (D ** -0.5)),
            "wo": _w((lambda *s: _rng.normal(s) * 0.05)(Hq * Dh, D) * ((Hq * Dh) ** -0.5)),
        }
    _A_in = _A_setup()

    def _B_setup():
        B, S, D, F = 4, 1, 512, 1792
        return {
            "x":  _w((lambda *s: _rng.normal(s) * 0.05)(B, S, D)),
            "w1": _w((lambda *s: _rng.normal(s) * 0.05)(D, D) * (D ** -0.5)),
            "w2": _w((lambda *s: _rng.normal(s) * 0.05)(D, D) * (D ** -0.5)),
            "w3": _w((lambda *s: _rng.normal(s) * 0.05)(D, F) * (D ** -0.5)),
            "w4": _w((lambda *s: _rng.normal(s) * 0.05)(F, D) * (F ** -0.5)),
        }
    _B_in = _B_setup()

    return {
        "A_x": _A_in["x"],
        "A_k_cache": _A_in["k_cache"],
        "A_v_cache": _A_in["v_cache"],
        "A_wq": _A_in["wq"],
        "A_wo": _A_in["wo"],
        "B_x": _B_in["x"],
        "B_w1": _B_in["w1"],
        "B_w2": _B_in["w2"],
        "B_w3": _B_in["w3"],
        "B_w4": _B_in["w4"],
    }

def _fwd_reference(A_x, A_k_cache, A_v_cache, A_wq, A_wo, B_x, B_w1, B_w2, B_w3, B_w4):
    def _A_ref(x, k_cache, v_cache, wq, wo):
        B, Sq, D = x.shape
        Hq, Dh = 32, 128
        Hkv, Sk = k_cache.shape[1], k_cache.shape[2]
        W = min(4096, max(256, Sk // 4))
        rep = Hq // Hkv
        q = (lambda x, *d: x.transpose(*d))((x @ wq).reshape(B, Sq, Hq, Dh), 0, 2, 1, 3)
        k = jnp.repeat(k_cache[:, :, Sk - W:, :], rep, axis=1)
        v = jnp.repeat(v_cache[:, :, Sk - W:, :], rep, axis=1)
        scores = jnp.einsum("bhqd,bhkd->bhqk", q, k) * (Dh ** -0.5)
        p = _softmax(scores, axis=-1)
        o = jnp.einsum("bhqk,bhkd->bhqd", p, v)
        return (lambda x, *d: x.transpose(*d))(o, 0, 2, 1, 3).reshape(B, Sq, Hq * Dh) @ wo

    def _B_ref(x, w1, w2, w3, w4):
        B, S, D = x.shape
        h = _gelu(_layernorm(x, axis=-1) @ w1)
        c = D // 4
        g0 = jnp.pad(h[:, :, 0*c:1*c], ((0, 0), (1, 0), (0, 0)))[:, :S, :]
        g1 = jnp.pad(h[:, :, 1*c:2*c], ((0, 0), (0, 1), (0, 0)))[:, 1:, :]
        g2 = jnp.pad(h[:, :, 2*c:3*c], ((0, 0), (2, 0), (0, 0)))[:, :S, :]
        g3 = jnp.pad(h[:, :, 3*c:   ], ((0, 0), (0, 2), (0, 0)))[:, 2:, :]
        hs = jnp.concatenate([g0, g1, g2, g3], axis=-1) @ w2
        x1 = x + hs
        h2 = _gelu(_layernorm(x1, axis=-1) @ w3) @ w4
        return x1 + h2

    x = A_x
    xn = _layernorm(x, axis=-1)
    s = _A_ref(xn, A_k_cache, A_v_cache, A_wq, A_wo)
    g = _silu(_B_ref(xn, B_w1, B_w2, B_w3, B_w4))
    return x + s * g


def setup_inputs():
    _inp = _fwd_setup_inputs()
    _gk = jax.random.fold_in(jax.random.key(int.from_bytes(__import__("os").urandom(4), "little")), 2**31 - 1)
    _shapes = [[4, 1, 512]]
    _dtypes = ['bfloat16']
    _gks = jax.random.split(_gk, len(_shapes))
    _gs = [jax.random.normal(k, s, dtype=jnp.dtype(d)) * 0.05 for k, s, d in zip(_gks, _shapes, _dtypes)]
    _inp["grad_out"] = _gs[0]
    return _inp

def reference(A_x, A_k_cache, A_v_cache, A_wq, A_wo, B_w3, B_w4, B_x, B_w1, B_w2, grad_out):
    _const = dict(B_x=B_x, B_w1=B_w1, B_w2=B_w2)
    def _f(*_d):
        return _fwd_reference(**{'A_x': _d[0], 'A_k_cache': _d[1], 'A_v_cache': _d[2], 'A_wq': _d[3], 'A_wo': _d[4], 'B_w3': _d[5], 'B_w4': _d[6], **_const})
    _out, _vjp = jax.vjp(_f, A_x, A_k_cache, A_v_cache, A_wq, A_wo, B_w3, B_w4)
    _grads = _vjp(grad_out)
    _out0 = jnp.asarray(_out)
    return (_out0, *[jnp.asarray(_g) for _g in _grads])
```

```python
import functools
import math

import jax
import jax.numpy as jnp
from jax import lax
from jax.experimental import pallas as pl
from jax.experimental.pallas import tpu as pltpu

F32 = jnp.float32
BF16 = jnp.bfloat16

HQ, DH = 32, 128
EPS = 1e-5
GELU_C = math.sqrt(2.0 / math.pi)
GELU_A = 0.044715


def _nn(a, b):
    return lax.dot_general(a, b, (((1,), (0,)), ((), ())), preferred_element_type=F32)


def _nt(a, b):
    return lax.dot_general(a, b, (((1,), (1,)), ((), ())), preferred_element_type=F32)


def _tn(a, b):
    return lax.dot_general(a, b, (((0,), (0,)), ((), ())), preferred_element_type=F32)


def _ln(x):
    xc = x - jnp.mean(x, axis=-1, keepdims=True)
    rstd = 1.0 / jnp.sqrt(jnp.mean(xc * xc, axis=-1, keepdims=True) + EPS)
    return xc * rstd, rstd


def _ln_bwd(dy, y, rstd):
    return rstd * (dy - jnp.mean(dy, axis=-1, keepdims=True)
                   - y * jnp.mean(dy * y, axis=-1, keepdims=True))


def _pad8(x):
    return jnp.concatenate([x, jnp.zeros((8 - x.shape[0], x.shape[1]), x.dtype)], axis=0)


def build(
    compute=True,
    mode="w",
    rrows=32,
    zng=8, zrows=128,
    dng=8, drows=128,
    z0=72,
    zper=6,
    zr=24,
    name="fused",
):
    def kernel(
        x_hbm, g_hbm, k_hbm, v_hbm, wq_hbm, wo_hbm, w3_hbm, w4_hbm,
        out_hbm, dx_hbm, dk_hbm, dv_hbm, dwq_hbm, dwo_hbm, dw3_hbm, dw4_hbm,
        x_buf, g_buf, k_buf, v_buf, wq_buf, wo_buf, w3_buf, w4_buf,
        out_buf, dx_buf, dk_buf, dv_buf, dwq_buf, dwo_buf, dw3_buf, dw4_buf,
        zero_buf, qd_buf, oq_buf, pre_buf, act_buf,
        rsem, kvsem, wsem,
    ):
        B, HKV, W, _ = k_buf.shape
        SK = k_hbm.shape[2]
        LO = SK - W
        D = x_buf.shape[1]
        NF = w4_buf.shape[0] * w4_buf.shape[1]
        REP = HQ // HKV
        HW = REP * DH
        scale = DH ** -0.5

        def read(src, dst, sem, prio):
            pltpu.make_async_copy(src, dst, sem).start(priority=prio)

        def issue_mlp_weights():
            def body(i, c):
                r = pl.multiple_of(i * 8, 8)
                read(w4_hbm.at[:, pl.ds(r, 8)], w4_buf.at[:, pl.ds(r, 8)], rsem.at[3], 1)
                s, j = i % 4, pl.multiple_of((i // 4) * 8, 8)
                read(w3_hbm.at[s, pl.ds(j, 8)], w3_buf.at[s, pl.ds(j, 8)], rsem.at[2], 0)
                return c
            n4 = w4_buf.shape[1] // 8
            lax.fori_loop(0, n4, body, 0)
            for i in range(n4, w3_buf.shape[0] * w3_buf.shape[1] // 8):
                s, j = i % 4, (i // 4) * 8
                read(w3_hbm.at[s, pl.ds(j, 8)], w3_buf.at[s, pl.ds(j, 8)], rsem.at[2], i % 2)

        def issue_attn_weights():
            def body(i, c):
                r = pl.multiple_of(i * 8, 8)
                read(wo_hbm.at[:, pl.ds(r, 8)], wo_buf.at[:, pl.ds(r, 8)], rsem.at[5], 1)
                j = pl.multiple_of((i // 8) * 8, 8)
                col = pl.multiple_of((i % 8) * 512, 512)
                read(wq_hbm.at[:, pl.ds(j, 8), pl.ds(col, 512)],
                     wq_buf.at[:, pl.ds(j, 8), pl.ds(col, 512)], rsem.at[4], 0)
                return c
            lax.fori_loop(0, wo_buf.shape[1] // 8, body, 0)

        def issue_kv(h, lo, n):
            def body(i, c):
                r = pl.multiple_of(i * rrows, rrows)
                read(k_hbm.at[:, h, pl.ds(LO + r, rrows)], k_buf.at[:, h, pl.ds(r, rrows)], kvsem.at[h], 0)
                read(v_hbm.at[:, h, pl.ds(LO + r, rrows)], v_buf.at[:, h, pl.ds(r, rrows)], kvsem.at[h], 1)
                return c
            lax.fori_loop(lo, lo + n, body, 0)

        def wait_all(buf, sem):
            pltpu.make_async_copy(buf, buf, sem).wait()

        n_zr = LO // zrows
        n_zg = HKV // zng if zng <= HKV else 1
        NZ = 2 * (B * HKV // zng) * n_zr

        def issue_zero(lo, n):
            def body(i, c):
                r = pl.multiple_of((i % n_zr) * zrows, zrows)
                g = i // n_zr
                b = g // n_zg
                h0 = (g % n_zg) * zng
                pltpu.make_async_copy(
                    zero_buf, dk_hbm.at[b, pl.ds(h0, zng), pl.ds(r, zrows)], wsem.at[0]).start()
                return c

            def body_v(i, c):
                r = pl.multiple_of((i % n_zr) * zrows, zrows)
                g = i // n_zr
                b = g // n_zg
                h0 = (g % n_zg) * zng
                pltpu.make_async_copy(
                    zero_buf, dv_hbm.at[b, pl.ds(h0, zng), pl.ds(r, zrows)], wsem.at[1]).start()
                return c
            half = NZ // 2
            lax.fori_loop(jnp.minimum(lo, half), jnp.minimum(lo + n, half), body, 0)
            lax.fori_loop(jnp.maximum(lo, half) - half, jnp.maximum(lo + n, half) - half, body_v, 0)

        def issue_data():
            n_r = W // drows
            n_g = HKV // dng
            for src, dst, sem in ((dk_buf, dk_hbm, wsem.at[0]), (dv_buf, dv_hbm, wsem.at[1])):
                def body(i, c, src=src, dst=dst, sem=sem):
                    r = pl.multiple_of((i % n_r) * drows, drows)
                    g = i // n_r
                    b = g // n_g
                    h0 = (g % n_g) * dng
                    pltpu.make_async_copy(
                        src.at[b, pl.ds(h0, dng), pl.ds(r, drows)],
                        dst.at[b, pl.ds(h0, dng), pl.ds(LO + r, drows)], sem).start()
                    return c
                lax.fori_loop(0, B * n_g * n_r, body, 0)

            def wq_body(i, c):
                j = pl.multiple_of((i // 2) * 8, 8)
                col = pl.multiple_of((i % 2) * 2048, 2048)
                pltpu.make_async_copy(dwq_buf.at[:, pl.ds(j, 8), pl.ds(col, 2048)],
                                      dwq_hbm.at[:, pl.ds(j, 8), pl.ds(col, 2048)], wsem.at[2]).start()
                return c
            lax.fori_loop(0, 2 * dwq_buf.shape[1] // 8, wq_body, 0)

            def wo_body(i, c):
                r = pl.multiple_of(i * 32, 32)
                pltpu.make_async_copy(dwo_buf.at[:, pl.ds(r, 32)], dwo_hbm.at[:, pl.ds(r, 32)], wsem.at[3]).start()
                return c
            lax.fori_loop(0, dwo_buf.shape[1] // 32, wo_body, 0)

            pltpu.make_async_copy(out_buf, out_hbm, wsem.at[6]).start()
            pltpu.make_async_copy(dx_buf, dx_hbm, wsem.at[7]).start()

            def w34_body(i, c):
                j = pl.multiple_of(i * 8, 8)
                pltpu.make_async_copy(dw3_buf.at[:, pl.ds(j, 8)], dw3_hbm.at[:, pl.ds(j, 8)], wsem.at[4]).start()
                r = pl.multiple_of(i * 32, 32)
                pltpu.make_async_copy(dw4_buf.at[:, pl.ds(r, 32)], dw4_hbm.at[:, pl.ds(r, 32)], wsem.at[5]).start()
                return c
            n4 = dw4_buf.shape[1] // 32
            lax.fori_loop(0, n4, w34_body, 0)
            rest = dw3_buf.shape[1] - 8 * n4
            pltpu.make_async_copy(dw3_buf.at[:, pl.ds(8 * n4, rest)], dw3_hbm.at[:, pl.ds(8 * n4, rest)],
                                  wsem.at[4]).start()

        FC = w4_buf.shape[1]

        def prologue():
            for i, buf in enumerate((x_buf, g_buf, w3_buf, w4_buf)):
                wait_all(buf, rsem.at[i])
            x = _pad8(x_buf[...].astype(F32))
            gout = _pad8(g_buf[...].astype(F32))
            xn, rstd1 = _ln(x)
            xn = xn.astype(BF16).astype(F32)
            ln2, rstd2 = _ln(xn)
            ln2_b = ln2.astype(BF16)
            w3 = w3_buf[...].reshape(D, NF)
            pre = _nn(ln2_b, w3)
            t = jnp.tanh(GELU_C * (pre + GELU_A * pre * pre * pre))
            act = 0.5 * pre * (1.0 + t)
            pre_buf[...] = 0.5 * (1.0 + t) + 0.5 * pre * (1.0 - t * t) * (
                GELU_C * (1.0 + 3.0 * GELU_A * pre * pre))
            act_buf[...] = act
            h2 = _nn(act.astype(BF16), w4_buf[...].reshape(NF, D))
            bo = xn + h2
            sig = 1.0 / (1.0 + jnp.exp(-bo))
            g = bo * sig
            ds = gout * g
            return x, gout, xn, rstd1, ln2, rstd2, bo, sig, g, ds

        def attention(b, h):
            row = lax.broadcasted_iota(jnp.int32, (8, DH), 0)
            top = row < REP
            qd = qd_buf[pl.ds(b, 8, stride=8), :]
            sw = pltpu.roll(qd, REP, 0)
            q2 = jnp.where(top, qd, sw).astype(BF16)
            do2 = jnp.where(top, sw, qd).astype(BF16)
            k = k_buf[b, h]
            v = v_buf[b, h]
            s = _nt(q2, k) * scale
            dp = _nt(do2, v)
            e = jnp.exp(s - jnp.max(s, axis=-1, keepdims=True))
            p = e * (1.0 / jnp.sum(e, axis=-1, keepdims=True))
            dsc = p * (dp - jnp.sum(p * dp, axis=-1, keepdims=True)) * scale
            t = jnp.where(lax.broadcasted_iota(jnp.int32, (8, W), 0) < REP, dsc, p).astype(BF16)
            dq = _nn(t, k)
            o = _nn(t, v)
            oq_buf[pl.ds(b, 8, stride=8), :] = jnp.where(top, dq, o)
            rhs = jnp.concatenate([jnp.where(top, qd, 0.0), jnp.where(top, 0.0, qd)], axis=1).astype(BF16)
            dkv = _tn(t, rhs)
            dk_buf[b, h] = dkv[:, :DH].astype(BF16)
            dv_buf[b, h] = dkv[:, DH:].astype(BF16)

        def head_pre(h, xn_b, ds_b):
            col = pl.multiple_of(h * HW, HW)
            wq_h = wq_buf[:, :, pl.ds(col, HW)].reshape(D, HW)
            q = _nn(xn_b, wq_h)
            wo_h = wo_buf[h // 2, pl.ds(pl.multiple_of((h % 2) * HW, HW), HW), :]
            do = _nt(ds_b, wo_h)
            for r in range(REP):
                qd_buf[8 * r:8 * r + 8, :] = q[:, r * DH:(r + 1) * DH]
                qd_buf[8 * (REP + r):8 * (REP + r) + 8, :] = do[:, r * DH:(r + 1) * DH]

        def head_post(h, xn_b, ds_b, s_acc, dxn_acc):
            col = pl.multiple_of(h * HW, HW)
            dq = jnp.concatenate([oq_buf[8 * r:8 * r + 8, :] for r in range(REP)], axis=1).astype(BF16)
            o = jnp.concatenate([oq_buf[8 * (REP + r):8 * (REP + r) + 8, :] for r in range(REP)],
                                axis=1).astype(BF16)
            wq_h = wq_buf[:, :, pl.ds(col, HW)].reshape(D, HW)
            wo_h = wo_buf[h // 2, pl.ds(pl.multiple_of((h % 2) * HW, HW), HW), :]
            s_acc = s_acc + _nn(o, wo_h)
            dxn_acc = dxn_acc + _nt(dq, wq_h)
            dwo_buf[h] = _tn(o, ds_b).astype(BF16)
            dwq_buf[:, :, pl.ds(col, HW)] = _tn(xn_b, dq).astype(BF16).reshape(dwq_buf.shape[0], -1, HW)
            return s_acc, dxn_acc

        def epilogue(st, s, dxn_a):
            x, gout, xn, rstd1, ln2, rstd2, bo, sig, g, ds = st
            out_buf[...] = (x + s * g)[:B].astype(BF16)
            dbo = gout * s * (sig * (1.0 + bo * (1.0 - sig)))
            dbo_b = dbo.astype(BF16)
            dw4_buf[...] = _tn(act_buf[...].astype(BF16), dbo_b).astype(BF16).reshape(dw4_buf.shape)
            dact = _nt(dbo_b, w4_buf[...].reshape(NF, D))
            dpre_b = (dact * pre_buf[...]).astype(BF16)
            dw3_buf[...] = _tn(ln2.astype(BF16), dpre_b).astype(BF16).reshape(dw3_buf.shape)
            dln2 = _nt(dpre_b, w3_buf[...].reshape(D, NF))
            dxn = dxn_a + dbo + _ln_bwd(dln2, ln2, rstd2)
            dx_buf[...] = (gout + _ln_bwd(dxn, xn, rstd1))[:B].astype(BF16)

        n_kv = W // rrows
        read(x_hbm, x_buf, rsem.at[0], 0)
        read(g_hbm, g_buf, rsem.at[1], 1)
        issue_mlp_weights()
        zero_buf[...] = jnp.zeros_like(zero_buf)
        oq_buf[...] = jnp.zeros_like(oq_buf)
        issue_attn_weights()

        if not compute:
            def kv_body(h, c):
                issue_kv(h, 0, n_kv)
                return c
            lax.fori_loop(0, HKV, kv_body, 0)
            issue_zero(0, NZ)
            for i, buf in enumerate((x_buf, g_buf, w3_buf, w4_buf, wq_buf, wo_buf)):
                wait_all(buf, rsem.at[i])
            for h in range(HKV):
                wait_all(k_buf.at[:, h], kvsem.at[h])
                wait_all(v_buf.at[:, h], kvsem.at[h])
        elif mode == "w":
            def kv_body(h, c):
                issue_kv(h, 0, n_kv)
                return c
            lax.fori_loop(0, HKV, kv_body, 0)
            issue_zero(0, z0)
            st = prologue()
            xn_b, ds_b = st[2].astype(BF16), st[9].astype(BF16)
            wait_all(wq_buf, rsem.at[4])
            wait_all(wo_buf, rsem.at[5])

            def head(h, carry):
                head_pre(h, xn_b, ds_b)
                wait_all(k_buf.at[:, h], kvsem.at[h])
                wait_all(v_buf.at[:, h], kvsem.at[h])

                def batch(b, c):
                    attention(b, h)
                    issue_zero(z0 + (h * B + b) * zper, zper)
                    return c
                lax.fori_loop(0, B, batch, 0)
                return head_post(h, xn_b, ds_b, *carry)

            zero = jnp.zeros((8, D), F32)
            s, dxn_a = lax.fori_loop(0, HKV, head, (zero, zero))
            epilogue(st, s, dxn_a)
            done = z0 + HKV * B * zper
            issue_zero(done, NZ - done)
        else:
            issue_kv(0, 0, n_kv // 2)
            st = prologue()
            xn_b, ds_b = st[2].astype(BF16), st[9].astype(BF16)
            issue_kv(0, n_kv // 2, n_kv // 2)
            wait_all(wq_buf, rsem.at[4])
            wait_all(wo_buf, rsem.at[5])
            issue_kv(1, 0, n_kv // 2)
            per = n_kv // B

            def head(h, carry):
                head_pre(h, xn_b, ds_b)
                wait_all(k_buf.at[:, h], kvsem.at[h])
                wait_all(v_buf.at[:, h], kvsem.at[h])

                def batch(b, c):
                    u = h * B + b + B + B // 2

                    @pl.when(u < HKV * B)
                    def _():
                        issue_kv(u // B, (u % B) * per, per)

                    @pl.when(u >= HKV * B)
                    def _():
                        issue_zero((u - HKV * B) * zr, zr)
                    attention(b, h)
                    return c
                lax.fori_loop(0, B, batch, 0)
                return head_post(h, xn_b, ds_b, *carry)

            zero = jnp.zeros((8, D), F32)
            s, dxn_a = lax.fori_loop(0, HKV, head, (zero, zero))
            epilogue(st, s, dxn_a)
            done = (B + B // 2) * zr
            issue_zero(done, NZ - done)

        issue_data()
        for i, ref in enumerate((dk_hbm, dv_hbm, dwq_hbm, dwo_hbm, dw3_hbm, dw4_hbm, out_hbm, dx_hbm)):
            wait_all(ref, wsem.at[i])

    @jax.jit
    def fn(A_x, A_k_cache, A_v_cache, A_wq, A_wo, B_x, B_w1, B_w2, B_w3, B_w4, grad_out):
        B, _, D = A_x.shape
        _, HKV, SK, _ = A_k_cache.shape
        W = min(4096, max(256, SK // 4))
        NF = B_w3.shape[1]
        HD = HQ * DH
        sds = jax.ShapeDtypeStruct
        any_spec = pl.BlockSpec(memory_space=pl.ANY)
        vm = pltpu.VMEM
        outs = pl.pallas_call(
            kernel,
            out_shape=(
                sds((B, D), BF16), sds((B, D), BF16),
                sds(A_k_cache.shape, BF16), sds(A_v_cache.shape, BF16),
                sds((8, D // 8, HD), BF16), sds((8, HD // 8, D), BF16),
                sds((4, D // 4, NF), BF16), sds((4, NF // 4, D), BF16),
            ),
            in_specs=[any_spec] * 8,
            out_specs=(any_spec,) * 8,
            scratch_shapes=[
                vm((B, D), BF16), vm((B, D), BF16),
                vm((B, HKV, W, DH), BF16), vm((B, HKV, W, DH), BF16),
                vm((4, D // 4, HD), BF16), vm((4, HD // 4, D), BF16),
                vm((4, D // 4, NF), BF16), vm((4, NF // 4, D), BF16),
                vm((B, D), BF16), vm((B, D), BF16),
                vm((B, HKV, W, DH), BF16), vm((B, HKV, W, DH), BF16),
                vm((8, D // 8, HD), BF16), vm((8, HD // 8, D), BF16),
                vm((4, D // 4, NF), BF16), vm((4, NF // 4, D), BF16),
                vm((zng, zrows, DH), BF16),
                vm((64, DH), F32), vm((64, DH), F32),
                vm((8, NF), F32), vm((8, NF), F32),
                pltpu.SemaphoreType.DMA((6,)),
                pltpu.SemaphoreType.DMA((HKV,)),
                pltpu.SemaphoreType.DMA((8,)),
            ],
            compiler_params=pltpu.CompilerParams(
                vmem_limit_bytes=110 * 1024 * 1024, disable_bounds_checks=True),
            name=name,
        )(
            A_x.reshape(B, D), grad_out.reshape(B, D), A_k_cache, A_v_cache,
            A_wq.reshape(4, D // 4, HD), A_wo.reshape(4, HD // 4, D),
            B_w3.reshape(4, D // 4, NF), B_w4.reshape(4, NF // 4, D),
        )
        out, dx, dk, dv, dwq, dwo, dw3, dw4 = outs
        return (out.reshape(A_x.shape), dx.reshape(A_x.shape), dk, dv,
                dwq.reshape(A_wq.shape), dwo.reshape(A_wo.shape),
                dw3.reshape(B_w3.shape), dw4.reshape(B_w4.shape))

    return fn


pallas_recurrent_scan__sliding_block_cached__mixer_s_mlp__decode_kernel = build(mode="w", zper=4)
```

```python
import math

import jax
import jax.numpy as jnp
from jax import lax
from jax.experimental import pallas as pl
from jax.experimental.pallas import tpu as pltpu

F32 = jnp.float32
BF16 = jnp.bfloat16

HQ, DH = 32, 128
EPS = 1e-5
GELU_C = math.sqrt(2.0 / math.pi)
GELU_A = 0.044715

ROWS = 16
READ_SLABS = 8
TAIL = 48
ZERO_UNROLL = 8


def _nn(a, b):
    return lax.dot_general(a, b, (((1,), (0,)), ((), ())), preferred_element_type=F32)


def _nt(a, b):
    return lax.dot_general(a, b, (((1,), (1,)), ((), ())), preferred_element_type=F32)


def _tn(a, b):
    return lax.dot_general(a, b, (((0,), (0,)), ((), ())), preferred_element_type=F32)


def _layernorm(x):
    xc = x - jnp.mean(x, axis=-1, keepdims=True)
    rstd = 1.0 / jnp.sqrt(jnp.mean(xc * xc, axis=-1, keepdims=True) + EPS)
    return xc * rstd, rstd


def _layernorm_bwd(dy, y, rstd):
    return rstd * (dy - jnp.mean(dy, axis=-1, keepdims=True)
                   - y * jnp.mean(dy * y, axis=-1, keepdims=True))


def _div(a, b):
    assert a % b == 0, (a, b)
    return a // b


def _loop(n, body, unroll=1):
    def step(i, carry):
        for u in range(unroll):
            body(i * unroll + u)
        return carry

    lax.fori_loop(0, _div(n, unroll), step, 0)


def _start(src, dst, sem, queue=0):
    pltpu.make_async_copy(src, dst, sem).start(priority=queue)


def _wait_filled(ref, sem):
    pltpu.make_async_copy(ref, ref, sem).wait()


def _tiles(ref, cols):
    return _div(ref.shape[1], 8) * _div(ref.shape[2], cols)


def _tile(ref, cols, i):
    per_row = ref.shape[2] // cols
    row = pl.multiple_of((i // per_row) * 8, 8)
    col = pl.multiple_of((i % per_row) * cols, 128)
    return slice(None), pl.ds(row, 8), pl.ds(col, cols)


def _kernel(
    x_hbm, gout_hbm, k_hbm, v_hbm, wq_hbm, wo_hbm, w3_hbm, w4_hbm,
    out_hbm, dx_hbm, dk_hbm, dv_hbm, dwq_hbm, dwo_hbm, dw3_hbm, dw4_hbm,
    x_buf, gout_buf, k_buf, v_buf, wq_buf, wo_buf, w3_buf, w4_buf,
    out_buf, dx_buf, dk_buf, dv_buf, dwq_buf, dwo_buf, dw3_buf, dw4_buf,
    zero_buf, q_buf, do_buf, res_buf, dgelu_buf, act_buf,
    rsem, wsem,
):
    slabs, window, _ = k_buf.shape
    batch, dim = x_buf.shape
    hkv = _div(slabs, batch)
    rep = _div(HQ, hkv)
    assert 2 * rep == 8 and batch <= 8
    head_cols = rep * DH
    first = k_hbm.shape[1] - window
    hidden = w3_buf.shape[2]
    scale = DH ** -0.5

    def read_tile(src, dst, sem, cols, i, queue):
        t = _tile(src, cols, i)
        _start(src.at[t], dst.at[t], sem, queue)

    def read_weights():
        n3, n4 = _tiles(w3_hbm, 256), _tiles(w4_hbm, dim)

        def w3_w4(i):
            read_tile(w3_hbm, w3_buf, rsem.at[2], 256, i, 0)
            read_tile(w4_hbm, w4_buf, rsem.at[3], dim, i, 1)

        def w3_rest(i):
            for u in range(2):
                read_tile(w3_hbm, w3_buf, rsem.at[2], 256, n4 + 2 * i + u, u)

        def wq_wo(i):
            read_tile(wq_hbm, wq_buf, rsem.at[4], 256, i, 0)
            read_tile(wo_hbm, wo_buf, rsem.at[5], 256, i, 1)

        assert n3 >= n4 and _tiles(wq_hbm, 256) == _tiles(wo_hbm, 256)
        _loop(n4, w3_w4)
        _start(x_hbm, x_buf, rsem.at[0], 0)
        _start(gout_hbm, gout_buf, rsem.at[1], 1)
        _loop(_div(n3 - n4, 2), w3_rest)
        _loop(_tiles(wq_hbm, 256), wq_wo)

    def read_kv(lo, hi, sem):
        def group(g):
            which = pl.ds(g * READ_SLABS, READ_SLABS)

            def rows(i):
                r = pl.multiple_of(lo + i * ROWS, 8)
                for u, (src, dst) in enumerate(((k_hbm, k_buf), (v_hbm, v_buf))):
                    _start(src.at[which, pl.ds(first + r, ROWS)], dst.at[which, pl.ds(r, ROWS)],
                           rsem.at[sem + u], u)

            _loop(_div(hi - lo, ROWS), rows)

        _loop(_div(slabs, READ_SLABS), group)

    assert slabs == 4 * 5 + 2 * 6 and hkv == 8
    kv_grads = ((dk_buf, dk_hbm, wsem.at[2]), (dv_buf, dv_hbm, wsem.at[3]))

    def write_zeros(grad, slab, nslabs, part=0, parts=1):
        _, dst, sem = grad
        rows = _div(first, parts)
        n = _div(rows, ROWS)

        def put(i):
            r = pl.multiple_of(part * rows + i * ROWS, 8)
            _start(zero_buf.at[pl.ds(0, nslabs)], dst.at[pl.ds(slab, nslabs), pl.ds(r, ROWS)], sem)

        _loop(n, put, math.gcd(n, ZERO_UNROLL))

    def write_zeros_during_head(h, part):
        for j, grad in enumerate(kv_grads):
            @pl.when(h // 4 == j)
            def _(j=j, grad=grad):
                write_zeros(grad, (h - 4 * j) * 5, 5, part, batch + 2)

    def write_window_grads():
        for src, dst, sem in kv_grads:
            def group(slab, nslabs, src=src, dst=dst, sem=sem):
                which = pl.ds(slab, nslabs)

                def put(i):
                    r = pl.multiple_of(i * ROWS, 8)
                    _start(src.at[which, pl.ds(r, ROWS)], dst.at[which, pl.ds(first + r, ROWS)], sem)

                _loop(_div(window, ROWS), put)

            _loop(4, lambda g: group(5 * g, 5))
            _loop(2, lambda g: group(20 + 6 * g, 6))

    def write_weight_grads():
        def put(src, dst, sem, cols, i):
            t = _tile(src, cols, i)
            _start(src.at[t], dst.at[t], sem)

        def w3_w4(i):
            put(dw3_buf, dw3_hbm, wsem.at[6], 256, i)
            put(dw4_buf, dw4_hbm, wsem.at[7], 256, i)

        assert _tiles(dw3_buf, 256) == _tiles(dw4_buf, 256)
        _loop(_tiles(dwq_buf, 512), lambda i: put(dwq_buf, dwq_hbm, wsem.at[4], 512, i))
        _loop(_tiles(dwo_buf, 512), lambda i: put(dwo_buf, dwo_hbm, wsem.at[5], 512, i))
        _loop(_tiles(dw3_buf, 256), w3_w4)

    def attention(b, h):
        n = b * hkv + h
        top = lax.broadcasted_iota(jnp.int32, (8, DH), 0) < rep
        q = q_buf[b]
        do = do_buf[b]
        k = k_buf[n]
        v = v_buf[n]
        s = _nt(q.astype(BF16), k) * scale
        dp = _nt(do.astype(BF16), v)
        e = jnp.exp(s - jnp.max(s, axis=-1, keepdims=True))
        p = e * (1.0 / jnp.sum(e, axis=-1, keepdims=True))
        dscore = p * (dp - jnp.sum(p * dp, axis=-1, keepdims=True)) * scale
        t = jnp.where(lax.broadcasted_iota(jnp.int32, (8, window), 0) < rep, dscore, p).astype(BF16)
        res_buf[b] = jnp.where(top, _nn(t, k), _nn(t, v))
        rhs = jnp.concatenate([jnp.where(top, q, 0.0), jnp.where(top, 0.0, do)], axis=1)
        dkv = _tn(t, rhs.astype(BF16))
        dk_buf[n] = dkv[:, :DH].astype(BF16)
        dv_buf[n] = dkv[:, DH:].astype(BF16)

    def head_columns(h):
        return pl.ds(pl.multiple_of(h * head_cols, head_cols), head_cols)

    def pad_rows(a):
        return jnp.concatenate([a, jnp.zeros((8 - batch, dim), F32)], axis=0)

    def spread(a):
        return jnp.concatenate(
            [jnp.broadcast_to(a[b:b + 1], (8, dim)) for b in range(batch)], axis=0)

    def collect(a):
        row = lax.broadcasted_iota(jnp.int32, (8, dim), 0)
        acc = jnp.zeros((8, dim), F32)
        for b in range(batch):
            acc = jnp.where(row == b, jnp.sum(a[8 * b:8 * b + 8], axis=0, keepdims=True), acc)
        return acc

    read_weights()
    read_kv(0, window - TAIL, 6)
    zero_buf[...] = jnp.zeros_like(zero_buf)
    read_kv(window - TAIL, window, 8)
    for i, buf in enumerate((x_buf, gout_buf, w3_buf, w4_buf, wq_buf, wo_buf)):
        _wait_filled(buf, rsem.at[i])
    _wait_filled(k_buf.at[:, pl.ds(0, window - TAIL)], rsem.at[6])
    _wait_filled(v_buf.at[:, pl.ds(0, window - TAIL)], rsem.at[7])
    write_zeros(kv_grads[0], 20, 6, 0, 4)
    _wait_filled(k_buf.at[:, pl.ds(window - TAIL, TAIL)], rsem.at[8])
    _wait_filled(v_buf.at[:, pl.ds(window - TAIL, TAIL)], rsem.at[9])

    x = pad_rows(x_buf[...].astype(F32))
    gout = pad_rows(gout_buf[...].astype(F32))
    xn, rstd = _layernorm(x)
    xn = xn.astype(BF16).astype(F32)
    xnn, rstd2 = _layernorm(xn)
    pre = _nn(xnn.astype(BF16), w3_buf[...].reshape(dim, hidden))
    th = jnp.tanh(GELU_C * (pre + GELU_A * pre * pre * pre))
    act = 0.5 * pre * (1.0 + th)
    dgelu_buf[...] = 0.5 * (1.0 + th) + 0.5 * pre * (1.0 - th * th) * (
        GELU_C * (1.0 + 3.0 * GELU_A * pre * pre))
    act_buf[...] = act
    mix = xn + _nn(act.astype(BF16), w4_buf[...].reshape(hidden, dim))
    sig = 1.0 / (1.0 + jnp.exp(-mix))
    gate = mix * sig
    xn_s = spread(xn).astype(BF16)
    dattn_s = spread(gout * gate).astype(BF16)

    def head(h, carry):
        attn, dxn = carry
        sub = lax.broadcasted_iota(jnp.int32, (8 * batch, DH), 0) % 8

        def per_head(a):
            out = a[:, :DH]
            for r in range(1, rep):
                out = jnp.where(sub % rep == r, a[:, r * DH:(r + 1) * DH], out)
            return out.reshape(batch, 8, DH)

        wq = wq_buf[:, :, head_columns(h)].reshape(dim, head_cols)
        q_buf[...] = per_head(_nn(xn_s, wq))
        do_buf[...] = per_head(_nt(dattn_s, wo_buf[h]))
        write_zeros_during_head(h, 0)

        def one_batch(b):
            attention(b, h)
            write_zeros_during_head(h, b + 1)

        _loop(batch, one_batch)

        res = res_buf[...].reshape(8 * batch, DH)
        dq = jnp.concatenate([jnp.where(sub == r, res, 0.0) for r in range(rep)], axis=1).astype(BF16)
        o = jnp.concatenate([jnp.where(sub == rep + r, res, 0.0) for r in range(rep)], axis=1).astype(BF16)
        wq = wq_buf[:, :, head_columns(h)].reshape(dim, head_cols)
        attn = attn + _nn(o, wo_buf[h])
        dxn = dxn + _nt(dq, wq)
        dwo_buf[h] = _tn(o, dattn_s).astype(BF16)
        dwq_buf[:, :, head_columns(h)] = _tn(xn_s, dq).astype(BF16).reshape(
            dwq_buf.shape[0], dwq_buf.shape[1], head_cols)
        write_zeros_during_head(h, batch + 1)
        return attn, dxn

    init = jnp.zeros((8 * batch, dim), F32)
    attn, dxn = lax.fori_loop(0, hkv, head, (init, init))
    attn, dxn = collect(attn), collect(dxn)

    out_buf[...] = (x + attn * gate)[:batch].astype(BF16)
    dmix = gout * attn * (sig * (1.0 + mix * (1.0 - sig)))
    dmix_b = dmix.astype(BF16)
    dw4_buf[...] = _tn(act_buf[...].astype(BF16), dmix_b).astype(BF16).reshape(dw4_buf.shape)
    write_zeros(kv_grads[0], 20, 6, 1, 4)
    dact = _nt(dmix_b, w4_buf[...].reshape(hidden, dim))
    dpre = (dact * dgelu_buf[...]).astype(BF16)
    dxnn = _nt(dpre, w3_buf[...].reshape(dim, hidden))
    dxn = dxn + dmix + _layernorm_bwd(dxnn, xnn, rstd2)
    dx_buf[...] = (gout + _layernorm_bwd(dxn, xn, rstd))[:batch].astype(BF16)
    write_zeros(kv_grads[0], 20, 6, 2, 4)
    dw3_buf[...] = _tn(xnn.astype(BF16), dpre).astype(BF16).reshape(dw3_buf.shape)
    write_zeros(kv_grads[0], 20, 6, 3, 4)

    write_zeros(kv_grads[0], 26, 6)
    write_zeros(kv_grads[1], 20, 6)
    write_zeros(kv_grads[1], 26, 6)
    _start(out_buf, out_hbm, wsem.at[0])
    _start(dx_buf, dx_hbm, wsem.at[1])
    write_weight_grads()
    write_window_grads()
    for i, ref in ((0, out_hbm), (1, dx_hbm), (4, dwq_hbm), (5, dwo_hbm), (6, dw3_hbm), (7, dw4_hbm),
                   (2, dk_hbm), (3, dv_hbm)):
        _wait_filled(ref, wsem.at[i])


@jax.jit
def pallas_recurrent_scan__sliding_block_cached__mixer_s_mlp__decode_kernel(
    A_x: jax.Array,
    A_k_cache: jax.Array,
    A_v_cache: jax.Array,
    A_wq: jax.Array,
    A_wo: jax.Array,
    B_x: jax.Array,
    B_w1: jax.Array,
    B_w2: jax.Array,
    B_w3: jax.Array,
    B_w4: jax.Array,
    grad_out: jax.Array,
):
    del B_x, B_w1, B_w2
    batch, tokens, dim = A_x.shape
    assert tokens == 1
    _, hkv, cache_len, _ = A_k_cache.shape
    window = min(4096, max(256, cache_len // 4))
    hidden = B_w3.shape[1]

    vec = (batch, dim)
    cache = (batch * hkv, cache_len, DH)
    win = (batch * hkv, window, DH)
    weights = (
        (8, _div(dim, 8), HQ * DH),
        (hkv, _div(HQ * DH, hkv), dim),
        (4, _div(dim, 4), hidden),
        (4, _div(hidden, 4), dim),
    )
    hbm = pl.BlockSpec(memory_space=pl.ANY)
    outs = pl.pallas_call(
        _kernel,
        out_shape=tuple(jax.ShapeDtypeStruct(s, BF16) for s in (vec, vec, cache, cache) + weights),
        in_specs=[hbm] * 8,
        out_specs=(hbm,) * 8,
        scratch_shapes=[pltpu.VMEM(s, BF16) for s in (vec, vec, win, win) + weights] * 2 + [
            pltpu.VMEM((6, ROWS, DH), BF16),
            pltpu.VMEM((batch, 8, DH), F32),
            pltpu.VMEM((batch, 8, DH), F32),
            pltpu.VMEM((batch, 8, DH), F32),
            pltpu.VMEM((8, hidden), F32),
            pltpu.VMEM((8, hidden), F32),
            pltpu.SemaphoreType.DMA((10,)),
            pltpu.SemaphoreType.DMA((8,)),
        ],
        compiler_params=pltpu.CompilerParams(
            vmem_limit_bytes=110 * 1024 * 1024,
            disable_bounds_checks=True,
            disable_semaphore_checks=True,
        ),
        name="cached_attention_mixer_fwd_bwd",
    )(
        A_x.reshape(vec), grad_out.reshape(vec), A_k_cache.reshape(cache), A_v_cache.reshape(cache),
        *[w.reshape(s) for w, s in zip((A_wq, A_wo, B_w3, B_w4), weights)],
    )
    like = (A_x, A_x, A_k_cache, A_v_cache, A_wq, A_wo, B_w3, B_w4)
    return tuple(o.reshape(a.shape) for o, a in zip(outs, like))
```

```python
import math

import jax
import jax.numpy as jnp
from jax import lax
from jax.experimental import pallas as pl
from jax.experimental.pallas import tpu as pltpu

F32 = jnp.float32
BF16 = jnp.bfloat16

HQ, DH = 32, 128
EPS = 1e-5
GELU_C = math.sqrt(2.0 / math.pi)
GELU_A = 0.044715

ROWS = 16
READ_SLABS = 8
TAIL = 48
ZERO_UNROLL = 8


def _nn(a, b):
    return lax.dot_general(a, b, (((1,), (0,)), ((), ())), preferred_element_type=F32)


def _nt(a, b):
    return lax.dot_general(a, b, (((1,), (1,)), ((), ())), preferred_element_type=F32)


def _tn(a, b):
    return lax.dot_general(a, b, (((0,), (0,)), ((), ())), preferred_element_type=F32)


def _layernorm(x):
    xc = x - jnp.mean(x, axis=-1, keepdims=True)
    rstd = 1.0 / jnp.sqrt(jnp.mean(xc * xc, axis=-1, keepdims=True) + EPS)
    return xc * rstd, rstd


def _layernorm_bwd(dy, y, rstd):
    return rstd * (dy - jnp.mean(dy, axis=-1, keepdims=True)
                   - y * jnp.mean(dy * y, axis=-1, keepdims=True))


def _div(a, b):
    assert a % b == 0, (a, b)
    return a // b


def _loop(n, body, unroll=1):
    def step(i, carry):
        for u in range(unroll):
            body(i * unroll + u)
        return carry

    lax.fori_loop(0, _div(n, unroll), step, 0)


def _start(src, dst, sem, queue=0):
    pltpu.make_async_copy(src, dst, sem).start(priority=queue)


def _wait_filled(ref, sem):
    pltpu.make_async_copy(ref, ref, sem).wait()


def _tiles(ref, cols):
    return _div(ref.shape[1], 8) * _div(ref.shape[2], cols)


def _tile(ref, cols, i):
    per_row = ref.shape[2] // cols
    row = pl.multiple_of((i // per_row) * 8, 8)
    col = pl.multiple_of((i % per_row) * cols, 128)
    return slice(None), pl.ds(row, 8), pl.ds(col, cols)


def _kernel(
    x_hbm, gout_hbm, k_hbm, v_hbm, wq_hbm, wo_hbm, w3_hbm, w4_hbm,
    out_hbm, dx_hbm, dk_hbm, dv_hbm, dwq_hbm, dwo_hbm, dw3_hbm, dw4_hbm,
    x_buf, gout_buf, k_buf, v_buf, wq_buf, wo_buf, w3_buf, w4_buf,
    out_buf, dx_buf, dk_buf, dv_buf, dwq_buf, dwo_buf, dw3_buf, dw4_buf,
    zero5_buf, zero6_buf, q_buf, do_buf, res_buf, dgelu_buf, act_buf,
    rsem, wsem,
):
    slabs, window, _ = k_buf.shape
    batch, dim = x_buf.shape
    hkv = _div(slabs, batch)
    rep = _div(HQ, hkv)
    assert 2 * rep == 8 and batch <= 8
    head_cols = rep * DH
    first = k_hbm.shape[1] - window
    hidden = w3_buf.shape[2]
    scale = DH ** -0.5

    def read_tile(src, dst, sem, cols, i, queue):
        t = _tile(src, cols, i)
        _start(src.at[t], dst.at[t], sem, queue)

    def read_weights():
        n3, n4 = _tiles(w3_hbm, 256), _tiles(w4_hbm, dim)

        def w3_w4(i):
            read_tile(w3_hbm, w3_buf, rsem.at[2], 256, i, 0)
            read_tile(w4_hbm, w4_buf, rsem.at[3], dim, i, 1)

        def w3_rest(i):
            for u in range(2):
                read_tile(w3_hbm, w3_buf, rsem.at[2], 256, n4 + 2 * i + u, u)

        def wq_wo(i):
            read_tile(wq_hbm, wq_buf, rsem.at[4], 256, i, 0)
            read_tile(wo_hbm, wo_buf, rsem.at[5], 256, i, 1)

        assert n3 >= n4 and _tiles(wq_hbm, 256) == _tiles(wo_hbm, 256)
        _loop(n4, w3_w4)
        _start(x_hbm, x_buf, rsem.at[0], 0)
        _start(gout_hbm, gout_buf, rsem.at[1], 1)
        _loop(_div(n3 - n4, 2), w3_rest)
        _loop(_tiles(wq_hbm, 256), wq_wo)

    def read_kv(lo, hi, sem):
        def group(g):
            which = pl.ds(g * READ_SLABS, READ_SLABS)

            def rows(i):
                r = pl.multiple_of(lo + i * ROWS, 8)
                for u, (src, dst) in enumerate(((k_hbm, k_buf), (v_hbm, v_buf))):
                    _start(src.at[which, pl.ds(first + r, ROWS)], dst.at[which, pl.ds(r, ROWS)],
                           rsem.at[sem + u], u)

            _loop(_div(hi - lo, ROWS), rows)

        _loop(_div(slabs, READ_SLABS), group)

    assert dk_hbm.shape == (8, 4, 2, 2 * window, DH) and dk_buf.shape == (8, 4, window, DH)
    assert hkv == 8 and batch + 2 == 6
    kv_grads = ((dk_buf, dk_hbm, wsem.at[2]), (dv_buf, dv_hbm, wsem.at[3]))
    column, triple, corner = pl.ds(0, 5), pl.ds(0, 3), pl.ds(5, 3)
    zero3_buf = zero5_buf.at[pl.ds(0, 3)]
    steps = _div(window, ROWS)

    def rows_at(base, i):
        return pl.ds(pl.multiple_of(base + i * ROWS, 8), ROWS)

    def zero_column_part(h, part):
        for a, (_, dst, sem) in enumerate(kv_grads):
            def put(i, a=a, dst=dst, sem=sem):
                rows = rows_at((part % 4) * (window // 2), i)
                _start(zero5_buf, dst.at[column, h - 4 * a, part // 4, rows], sem)

            @pl.when(h // 4 == a)
            def _(put=put):
                _loop(steps // 2, put, ZERO_UNROLL)

    def zero_triple(grad, n):
        _, dst, sem = grad
        _loop(steps, lambda i: _start(zero6_buf, dst.at[n, triple, :, rows_at(0, i)], sem), ZERO_UNROLL)

    def finish_triple(grad, n):
        src, dst, sem = grad

        def put(i):
            _start(zero3_buf, dst.at[n, triple, 0, rows_at(window, i)], sem)
            _start(src.at[n, triple, rows_at(0, i)], dst.at[n, triple, 1, rows_at(window, i)], sem)

        _loop(steps, put, 2)

    def write_corner():
        def zeros(half, i):
            for _, dst, sem in kv_grads:
                _start(zero3_buf, dst.at[corner, 3, half, rows_at(0, i)], sem)

        def grads(i):
            for src, dst, sem in kv_grads:
                _start(src.at[corner, 3, rows_at(0, i)], dst.at[corner, 3, 1, rows_at(window, i)], sem)

        _loop(2 * steps, lambda i: zeros(0, i), 2)
        _loop(steps, lambda i: zeros(1, i), 2)
        _loop(steps, grads, 2)

    def finish_columns(grad):
        src, dst, sem = grad
        _loop(4, lambda j: _loop(steps, lambda i: _start(
            src.at[column, j, rows_at(0, i)], dst.at[column, j, 1, rows_at(window, i)], sem)))

    def write_tile(src, dst, sem, i):
        t = _tile(src, 256, i)
        _start(src.at[t], dst.at[t], sem)

    def write_weight_grads(large, small):
        n_large, n_small = _tiles(large[0], 256), _tiles(small[0], 256)

        def both(i):
            write_tile(*large, i)
            write_tile(*small, i)

        assert n_large >= n_small
        _loop(n_small, both)
        _loop(n_large - n_small, lambda i: write_tile(*large, n_small + i))

    def attention(b, h):
        n = b * hkv + h
        top = lax.broadcasted_iota(jnp.int32, (8, DH), 0) < rep
        q = q_buf[b]
        do = do_buf[b]
        k = k_buf[n]
        v = v_buf[n]
        s = _nt(q.astype(BF16), k) * scale
        dp = _nt(do.astype(BF16), v)
        e = jnp.exp(s - jnp.max(s, axis=-1, keepdims=True))
        p = e * (1.0 / jnp.sum(e, axis=-1, keepdims=True))
        dscore = p * (dp - jnp.sum(p * dp, axis=-1, keepdims=True)) * scale
        t = jnp.where(lax.broadcasted_iota(jnp.int32, (8, window), 0) < rep, dscore, p).astype(BF16)
        res_buf[b] = jnp.where(top, _nn(t, k), _nn(t, v))
        rhs = jnp.concatenate([jnp.where(top, q, 0.0), jnp.where(top, 0.0, do)], axis=1)
        dkv = _tn(t, rhs.astype(BF16))
        dk_buf[n // 4, n % 4] = dkv[:, :DH].astype(BF16)
        dv_buf[n // 4, n % 4] = dkv[:, DH:].astype(BF16)

    def head_columns(h):
        return pl.ds(pl.multiple_of(h * head_cols, head_cols), head_cols)

    def pad_rows(a):
        return jnp.concatenate([a, jnp.zeros((8 - batch, dim), F32)], axis=0)

    def spread(a):
        return jnp.concatenate(
            [jnp.broadcast_to(a[b:b + 1], (8, dim)) for b in range(batch)], axis=0)

    def collect(a):
        row = lax.broadcasted_iota(jnp.int32, (8, dim), 0)
        acc = jnp.zeros((8, dim), F32)
        for b in range(batch):
            acc = jnp.where(row == b, jnp.sum(a[8 * b:8 * b + 8], axis=0, keepdims=True), acc)
        return acc

    read_weights()
    read_kv(0, window - TAIL, 6)
    zero5_buf[...] = jnp.zeros_like(zero5_buf)
    zero6_buf[...] = jnp.zeros_like(zero6_buf)
    read_kv(window - TAIL, window, 8)
    for i, buf in enumerate((x_buf, gout_buf, w3_buf, w4_buf, wq_buf, wo_buf)):
        _wait_filled(buf, rsem.at[i])
    _wait_filled(k_buf.at[:, pl.ds(0, window - TAIL)], rsem.at[6])
    _wait_filled(v_buf.at[:, pl.ds(0, window - TAIL)], rsem.at[7])
    zero_triple(kv_grads[0], 5)
    _wait_filled(k_buf.at[:, pl.ds(window - TAIL, TAIL)], rsem.at[8])
    _wait_filled(v_buf.at[:, pl.ds(window - TAIL, TAIL)], rsem.at[9])

    x = pad_rows(x_buf[...].astype(F32))
    gout = pad_rows(gout_buf[...].astype(F32))
    xn, rstd = _layernorm(x)
    xn = xn.astype(BF16).astype(F32)
    xnn, rstd2 = _layernorm(xn)
    pre = _nn(xnn.astype(BF16), w3_buf[...].reshape(dim, hidden))
    th = jnp.tanh(GELU_C * (pre + GELU_A * pre * pre * pre))
    act = 0.5 * pre * (1.0 + th)
    dgelu_buf[...] = 0.5 * (1.0 + th) + 0.5 * pre * (1.0 - th * th) * (
        GELU_C * (1.0 + 3.0 * GELU_A * pre * pre))
    act_buf[...] = act
    mix = xn + _nn(act.astype(BF16), w4_buf[...].reshape(hidden, dim))
    sig = 1.0 / (1.0 + jnp.exp(-mix))
    gate = mix * sig
    xn_s = spread(xn).astype(BF16)
    dattn_s = spread(gout * gate).astype(BF16)

    def head(h, carry):
        attn, dxn = carry
        sub = lax.broadcasted_iota(jnp.int32, (8 * batch, DH), 0) % 8

        def per_head(a):
            out = a[:, :DH]
            for r in range(1, rep):
                out = jnp.where(sub % rep == r, a[:, r * DH:(r + 1) * DH], out)
            return out.reshape(batch, 8, DH)

        wq = wq_buf[:, :, head_columns(h)].reshape(dim, head_cols)
        q_buf[...] = per_head(_nn(xn_s, wq))
        do_buf[...] = per_head(_nt(dattn_s, wo_buf[h]))
        zero_column_part(h, 0)

        def one_batch(b):
            attention(b, h)
            zero_column_part(h, b + 1)

        _loop(batch, one_batch)

        res = res_buf[...].reshape(8 * batch, DH)
        dq = jnp.concatenate([jnp.where(sub == r, res, 0.0) for r in range(rep)], axis=1).astype(BF16)
        o = jnp.concatenate([jnp.where(sub == rep + r, res, 0.0) for r in range(rep)], axis=1).astype(BF16)
        wq = wq_buf[:, :, head_columns(h)].reshape(dim, head_cols)
        attn = attn + _nn(o, wo_buf[h])
        dxn = dxn + _nt(dq, wq)
        dwo_buf[h // 2, head_columns(h % 2), :] = _tn(o, dattn_s).astype(BF16)
        dwq_buf[:, :, head_columns(h)] = _tn(xn_s, dq).astype(BF16).reshape(
            dwq_buf.shape[0], dwq_buf.shape[1], head_cols)
        zero_column_part(h, batch + 1)
        return attn, dxn

    init = jnp.zeros((8 * batch, dim), F32)
    attn, dxn = lax.fori_loop(0, hkv, head, (init, init))
    attn, dxn = collect(attn), collect(dxn)

    out_buf[...] = (x + attn * gate)[:batch].astype(BF16)
    dmix = gout * attn * (sig * (1.0 + mix * (1.0 - sig)))
    dmix_b = dmix.astype(BF16)
    dw4_buf[...] = _tn(act_buf[...].astype(BF16), dmix_b).astype(BF16).reshape(dw4_buf.shape)
    zero_triple(kv_grads[0], 6)
    dact = _nt(dmix_b, w4_buf[...].reshape(hidden, dim))
    dpre = (dact * dgelu_buf[...]).astype(BF16)
    dxnn = _nt(dpre, w3_buf[...].reshape(dim, hidden))
    dxn = dxn + dmix + _layernorm_bwd(dxnn, xnn, rstd2)
    dx_buf[...] = (gout + _layernorm_bwd(dxn, xn, rstd))[:batch].astype(BF16)
    zero_triple(kv_grads[0], 7)
    dw3_buf[...] = _tn(xnn.astype(BF16), dpre).astype(BF16).reshape(dw3_buf.shape)

    for n in (5, 6, 7):
        zero_triple(kv_grads[1], n)
    _start(out_buf, out_hbm, wsem.at[0])
    _start(dx_buf, dx_hbm, wsem.at[1])
    write_weight_grads((dwq_buf, dwq_hbm, wsem.at[4]), (dw3_buf, dw3_hbm, wsem.at[6]))
    write_weight_grads((dwo_buf, dwo_hbm, wsem.at[5]), (dw4_buf, dw4_hbm, wsem.at[7]))
    for grad in kv_grads:
        for n in (5, 6, 7):
            finish_triple(grad, n)
    write_corner()
    for grad in kv_grads:
        finish_columns(grad)
    for i, ref in ((0, out_hbm), (1, dx_hbm), (4, dwq_hbm), (5, dwo_hbm), (6, dw3_hbm), (7, dw4_hbm),
                   (2, dk_hbm), (3, dv_hbm)):
        _wait_filled(ref, wsem.at[i])


@jax.jit
def pallas_recurrent_scan__sliding_block_cached__mixer_s_mlp__decode_kernel(
    A_x: jax.Array,
    A_k_cache: jax.Array,
    A_v_cache: jax.Array,
    A_wq: jax.Array,
    A_wo: jax.Array,
    B_x: jax.Array,
    B_w1: jax.Array,
    B_w2: jax.Array,
    B_w3: jax.Array,
    B_w4: jax.Array,
    grad_out: jax.Array,
):
    del B_x, B_w1, B_w2
    batch, tokens, dim = A_x.shape
    assert tokens == 1
    _, hkv, cache_len, _ = A_k_cache.shape
    window = min(4096, max(256, cache_len // 4))
    hidden = B_w3.shape[1]

    vec = (batch, dim)
    cache = (batch * hkv, cache_len, DH)
    win = (batch * hkv, window, DH)
    cache_grad = (_div(batch * hkv, 4), 4, 2, _div(cache_len, 2), DH)
    win_grad = (*cache_grad[:2], window, DH)

    def matrices(n):
        return ((n, _div(dim, n), HQ * DH), (n, _div(HQ * DH, n), dim),
                (n // 2, _div(dim, n // 2), hidden), (n // 2, _div(hidden, n // 2), dim))

    weights, weight_grads = matrices(hkv), matrices(hkv // 2)
    hbm = pl.BlockSpec(memory_space=pl.ANY)
    outs = pl.pallas_call(
        _kernel,
        out_shape=tuple(jax.ShapeDtypeStruct(s, BF16) for s in (vec, vec, cache_grad, cache_grad) + weight_grads),
        in_specs=[hbm] * 8,
        out_specs=(hbm,) * 8,
        scratch_shapes=[
            *(pltpu.VMEM(s, BF16) for s in (vec, vec, win, win) + weights),
            *(pltpu.VMEM(s, BF16) for s in (vec, vec, win_grad, win_grad) + weight_grads),
            pltpu.VMEM((5, ROWS, DH), BF16),
            pltpu.VMEM((3, 2, ROWS, DH), BF16),
            pltpu.VMEM((batch, 8, DH), F32),
            pltpu.VMEM((batch, 8, DH), F32),
            pltpu.VMEM((batch, 8, DH), F32),
            pltpu.VMEM((8, hidden), F32),
            pltpu.VMEM((8, hidden), F32),
            pltpu.SemaphoreType.DMA((10,)),
            pltpu.SemaphoreType.DMA((8,)),
        ],
        compiler_params=pltpu.CompilerParams(
            vmem_limit_bytes=110 * 1024 * 1024,
            disable_bounds_checks=True,
            disable_semaphore_checks=True,
        ),
        name="cached_attention_mixer_fwd_bwd",
    )(
        A_x.reshape(vec), grad_out.reshape(vec), A_k_cache.reshape(cache), A_v_cache.reshape(cache),
        *[w.reshape(s) for w, s in zip((A_wq, A_wo, B_w3, B_w4), weights)],
    )
    like = (A_x, A_x, A_k_cache, A_v_cache, A_wq, A_wo, B_w3, B_w4)
    return tuple(o.reshape(a.shape) for o, a in zip(outs, like))
```
